```python
import jax
import jax.numpy as jnp

def _softmax(x, axis=-1):
    return jax.nn.softmax(x, axis=axis)
def _gelu(x):
    return jax.nn.gelu(x, approximate=True)
def _silu(x):
    return jax.nn.silu(x)
def _sigmoid(x):
    return jax.nn.sigmoid(x)
def _layernorm(x, axis=-1, eps=1e-5):
    m = jnp.mean(x, axis=axis, keepdims=True)
    v = jnp.var(x, axis=axis, keepdims=True)
    return (x - m) / jnp.sqrt(v + eps)
def _scatter_add(tgt, idx, src, axis=0):
    return tgt.at[idx].add(src)
def _segment_sum(src, seg, n):
    return jax.ops.segment_sum(src, seg, n)
class _Rng:
    def __init__(self, key):
        self._k = key
    def _next(self):
        self._k, sub = jax.random.split(self._k)
        return sub
    def normal(self, shape):
        return jax.random.normal(self._next(), shape, dtype=jnp.bfloat16)
    def randint(self, lo, hi, shape):
        return jax.random.randint(self._next(), shape, lo, hi, dtype=jnp.int32)
    def uniform(self, shape, lo=0.0, hi=1.0):
        return jax.random.uniform(self._next(), shape, jnp.bfloat16, lo, hi)
    def permutation(self, n):
        return jax.random.permutation(self._next(), n)


kernel_name = 'recurrent_scan__sliding_block_cached__dense_activation_gelu__decode'

def setup_inputs():
    _rng = _Rng(jax.random.key(int.from_bytes(__import__("os").urandom(4), "little")))
    _w = (lambda a: (lambda t: t.astype(jnp.bfloat16) if jnp.issubdtype(t.dtype, jnp.floating) else t)(jnp.asarray(a)))
    def _A_setup():
        B, Sq, D = 2, 1, 576
        Hq, Hkv, Sk, Dh = 32, 16, 32768, 128
        assert Hq % Hkv == 0, (Hq, Hkv)
        return {
            "x": _w((lambda *s: _rng.normal(s) * 0.05)(B, Sq, D)),
            "k_cache": _w((lambda *s: _rng.normal(s) * 0.05)(B, Hkv, Sk, Dh)),
            "v_cache": _w((lambda *s: _rng.normal(s) * 0.05)(B, Hkv, Sk, Dh)),
            "wq": _w((lambda *s: _rng.normal(s) * 0.05)(D, Hq * Dh) * (D ** -0.5)),
            "wo": _w((lambda *s: _rng.normal(s) * 0.05)(Hq * Dh, D) * ((Hq * Dh) ** -0.5)),
        }
    _A_in = _A_setup()

    def _B_setup():
        B, S, D, F = 2, 1, 576, 4608
        return {
            "x": _w((lambda *s: _rng.normal(s) * 0.05)(B, S, D)),
            "w1": _w((lambda *s: _rng.normal(s) * 0.05)(D, F) * (D ** -0.5)),
            "b1": _w((lambda *s: _rng.normal(s) * 0.05)(F) * 0.01),
            "w2": _w((lambda *s: _rng.normal(s) * 0.05)(F, D) * (F ** -0.5)),
            "b2": _w((lambda *s: _rng.normal(s) * 0.05)(D) * 0.01),
        }
    _B_in = _B_setup()

    return {
        "A_x": _A_in["x"],
        "A_k_cache": _A_in["k_cache"],
        "A_v_cache": _A_in["v_cache"],
        "A_wq": _A_in["wq"],
        "A_wo": _A_in["wo"],
        "B_x": _B_in["x"],
        "B_w1": _B_in["w1"],
        "B_b1": _B_in["b1"],
        "B_w2": _B_in["w2"],
        "B_b2": _B_in["b2"],
    }

def reference(A_x, A_k_cache, A_v_cache, A_wq, A_wo, B_x, B_w1, B_b1, B_w2, B_b2):
    def _A_ref(x, k_cache, v_cache, wq, wo):
        B, Sq, D = x.shape
        Hq, Dh = 32, 128
        Hkv, Sk = k_cache.shape[1], k_cache.shape[2]
        W = min(4096, max(256, Sk // 4))
        rep = Hq // Hkv
        q = (lambda x, *d: x.transpose(*d))((x @ wq).reshape(B, Sq, Hq, Dh), 0, 2, 1, 3)
        k = jnp.repeat(k_cache[:, :, Sk - W:, :], rep, axis=1)
        v = jnp.repeat(v_cache[:, :, Sk - W:, :], rep, axis=1)
        scores = jnp.einsum("bhqd,bhkd->bhqk", q, k) * (Dh ** -0.5)
        p = _softmax(scores, axis=-1)
        o = jnp.einsum("bhqk,bhkd->bhqd", p, v)
        return (lambda x, *d: x.transpose(*d))(o, 0, 2, 1, 3).reshape(B, Sq, Hq * Dh) @ wo

    def _B_ref(x, w1, b1, w2, b2):
        h = jnp.einsum("bsd,df->bsf", x, w1) + b1
        h = _gelu(h)
        return jnp.einsum("bsf,fd->bsd", h, w2) + b2

    x = A_x
    xn = _layernorm(x, axis=-1)
    s = _A_ref(xn, A_k_cache, A_v_cache, A_wq, A_wo)
    g = _silu(_B_ref(xn, B_w1, B_b1, B_w2, B_b2))
    return x + s * g
```

```python
import functools, math
import jax
import jax.numpy as jnp
import jax.experimental.pallas as pl
import jax.experimental.pallas.tpu as pltpu

CH = 128
NT = (((1,), (1,)), ((), ()))


def build(SR=512, R=8, AHEAD=4, unroll_inner=False, nobc=True, nocomp=False):
    def kern(x_hbm, k_hbm, v_hbm, wq_hbm, wot_hbm, w1_hbm, b1_hbm, w2t_hbm, b2_hbm, o_ref,
             xb, b1b, b2b, wqb, wob, w1b, w2b, kvb, q_scr, s_scr, h_scr, sem_s, sem_w, sem_kv):
        B, D = xb.shape
        _, HKV, SK, DH = k_hbm.shape
        W = min(4096, max(256, SK // 4))
        F = w1b.shape[1]
        NG = HKV // 2
        NS = W // SR
        CPS = SR // CH
        base = SK - W
        c_exp = (DH ** -0.5) * math.log2(math.e)
        blocks = [(r, min(128, D - r)) for r in range(0, D, 128)]
        NB = len(blocks)

        def issue_w(src, dst, sem, r0, nr, ns=4):
            half = src.shape[1] // 2
            tot = (nr // 8) * 2
            n = 0
            for i in range(tot // ns):
                for s in range(ns):
                    j = s * (tot // ns) + i
                    sl = (pl.ds(r0 + (j // 2) * 8, 8), pl.ds((j % 2) * half, half))
                    pltpu.make_async_copy(src.at[sl], dst.at[sl], sem).start(priority=n % 2)
                    n += 1

        def wait_w(dst, sem, r0, nr):
            d = dst.at[pl.ds(r0, nr)]
            pltpu.make_async_copy(d, d, sem).wait()

        def issue_kv(gk, gv, s, slot):
            n = 0
            for c in range(CPS):
                r = base + s * SR + c * CH
                if not isinstance(r, int):
                    r = pl.multiple_of(r, CH)
                for u in range(4):
                    for t, (src, g) in enumerate(((k_hbm, gk), (v_hbm, gv))):
                        if g is None:
                            continue
                        pr = t if (gk is not None and gv is not None) else n % 2
                        pltpu.make_async_copy(
                            src.at[u % 2, 2 * g + u // 2, pl.ds(r, CH), :],
                            kvb.at[slot, 4 * t + u, pl.ds(c * CH, CH), :],
                            sem_kv.at[slot]).start(priority=pr)
                        n += 1

        def wait_kv(slot, lo, n):
            d = kvb.at[slot, pl.ds(lo, n)]
            pltpu.make_async_copy(d, d, sem_kv.at[slot]).wait()

        WO_R = D // NS
        steps = []
        for i, (r0, nr) in enumerate(blocks):
            steps.append(functools.partial(issue_w, wq_hbm, wqb, sem_w.at[i], r0, nr))
        for i, (r0, nr) in enumerate(blocks):
            steps.append(functools.partial(issue_w, w1_hbm, w1b, sem_w.at[NB + i], r0, nr))
        def issue_e(s):
            issue_kv(0, None, s, s % R)
            issue_w(wot_hbm, wob, sem_w.at[3 * NB], s * WO_R, WO_R, ns=2)
        for s in range(NS):
            steps.append(functools.partial(issue_e, s))
        nA = len(steps)
        for s in range(AHEAD):
            steps.append(functools.partial(issue_kv, 1, 0, s, s % R))
        tail = []
        for s in range(NS):
            tail.append(functools.partial(issue_kv, None, NG - 1, s, s % R))
        for i, (r0, nr) in enumerate(blocks):
            tail.append(functools.partial(issue_w, w2t_hbm, w2b, sem_w.at[2 * NB + i], r0, nr))

        small = [pltpu.make_async_copy(a, b_, sem_s.at[i])
                 for i, (a, b_) in enumerate(((x_hbm, xb), (b1_hbm, b1b), (b2_hbm, b2b)))]
        small[0].start()
        for i in range(AHEAD):
            steps[i]()
            if i == 0:
                small[1].start()
                small[2].start()

        small[0].wait()
        row = jax.lax.broadcasted_iota(jnp.int32, (8, D), 0)
        xf = xb[...].astype(jnp.float32)
        x8 = jnp.where(row % 2 == 0, jnp.broadcast_to(xf[0:1], (8, D)), jnp.broadcast_to(xf[1:2], (8, D)))
        mu = jnp.mean(x8, axis=-1, keepdims=True)
        xc = x8 - mu
        var = jnp.mean(xc * xc, axis=-1, keepdims=True)
        xn = (xc / jnp.sqrt(var + 1e-5)).astype(jnp.bfloat16)

        si = 0
        q = None
        for i, (r0, nr) in enumerate(blocks):
            wait_w(wqb, sem_w.at[i], r0, nr)
            steps[si + AHEAD](); si += 1
            d = jnp.dot(xn[:, r0:r0 + nr], wqb[r0:r0 + nr, :], preferred_element_type=jnp.float32)
            q = d if q is None else q + d
        row128 = jax.lax.broadcasted_iota(jnp.int32, (8, DH), 0)
        for h in range(HKV):
            qa = q[:, 2 * h * DH:(2 * h + 1) * DH]
            qb = q[:, (2 * h + 1) * DH:(2 * h + 2) * DH]
            q_scr[h] = jnp.where(row128 % 4 < 2, qa, qb)
        hp = None
        for i, (r0, nr) in enumerate(blocks):
            wait_w(w1b, sem_w.at[NB + i], r0, nr)
            steps[si + AHEAD](); si += 1
            d = jnp.dot(xn[:, r0:r0 + nr], w1b[r0:r0 + nr, :], preferred_element_type=jnp.float32)
            hp = d if hp is None else hp + d
        small[1].wait()
        small[2].wait()
        hp = hp + b1b[...].astype(jnp.float32).reshape(1, F)
        h_scr[...] = jax.nn.gelu(hp, approximate=True)

        def qk_step(g, s, slot, mx):
            out = []
            for u in range(4):
                qh = q_scr[2 * g + u // 2].astype(jnp.bfloat16)
                sc = jax.lax.dot_general(qh, kvb[slot, u], NT, preferred_element_type=jnp.float32) * c_exp
                s_scr[g % 2, s, u] = sc
                m = mx[u]
                for j in range(SR // 128):
                    m = jnp.maximum(m, sc[:, j * 128:(j + 1) * 128])
                out.append(m)
            return out

        def pv_step(g, s, slot, m, l, acc):
            lo, ao = [], []
            for u in range(4):
                p = jnp.exp2(s_scr[g % 2, s, u] - m[u])
                ll = l[u]
                for j in range(SR // 128):
                    ll = ll + p[:, j * 128:(j + 1) * 128]
                lo.append(ll)
                ao.append(acc[u] + jnp.dot(p.astype(jnp.bfloat16), kvb[slot, 4 + u],
                                           preferred_element_type=jnp.float32))
            return lo, ao

        def finish(g, l, acc, so):
            o = [acc[u] / jnp.sum(l[u], axis=-1, keepdims=True) for u in range(4)]
            parts = []
            for hh in range(2):
                comb = jnp.where(row128 % 2 == 0, o[2 * hh], o[2 * hh + 1])
                parts.append(jnp.where(row128 < 2, comb, 0.0))
                parts.append(jnp.where((row128 >= 2) & (row128 < 4), comb, 0.0))
            lhs = jnp.concatenate(parts, axis=1).astype(jnp.bfloat16)
            c0 = g * 4 * DH
            if not isinstance(c0, int):
                c0 = pl.multiple_of(c0, 4 * DH)
            return so + jax.lax.dot_general(lhs, wob[:, pl.ds(c0, 4 * DH)], NT,
                                            preferred_element_type=jnp.float32)

        neg = [jnp.full((8, 128), -jnp.inf, jnp.float32)] * 4
        zero = [jnp.zeros((8, 128), jnp.float32)] * 4
        rowmax = lambda mx: [jnp.max(a, axis=-1, keepdims=True) for a in mx]

        mx = neg
        for s in range(NS):
            wait_kv(s % R, 0, 4)
            steps[si + AHEAD](); si += 1
            mx = qk_step(0, s, s % R, mx)
        wait_w(wob, sem_w.at[3 * NB], 0, D)

        def phase(g, carry):
            mx, so = carry
            m = rowmax(mx)

            def step(s, c):
                mx, l, acc = c
                slot = s % R
                wait_kv(slot, 0, 8)
                s2 = s + AHEAD
                g2 = g + s2 // NS
                s2 = s2 % NS

                @pl.when(g2 < NG)
                def _():
                    issue_kv(g2, g2 - 1, s2, s2 % R)

                @pl.when(g2 == NG)
                def _():
                    issue_kv(None, NG - 1, s2, s2 % R)

                if not nocomp:
                    mx = qk_step(g, s, slot, mx)
                    l, acc = pv_step(g - 1, s, slot, m, l, acc)
                return mx, l, acc

            mx, l, acc = jax.lax.fori_loop(0, NS, step, (neg, zero, zero), unroll=unroll_inner)
            return mx, finish(g - 1, l, acc, so)

        mx, so = jax.lax.fori_loop(1, NG, phase, (mx, jnp.zeros((8, D), jnp.float32)))
        m = rowmax(mx)
        l, acc = zero, zero
        ti = 0
        for s in range(NS):
            wait_kv(s % R, 4, 4)
            tail[ti + AHEAD](); ti += 1
            l, acc = pv_step(NG - 1, s, s % R, m, l, acc)
        so = finish(NG - 1, l, acc, so)
        hb = h_scr[...].astype(jnp.bfloat16)
        gs = []
        for i, (r0, nr) in enumerate(blocks):
            wait_w(w2b, sem_w.at[2 * NB + i], r0, nr)
            if ti + AHEAD < len(tail):
                tail[ti + AHEAD]()
            ti += 1
            gs.append(jax.lax.dot_general(hb, w2b[r0:r0 + nr, :], NT, preferred_element_type=jnp.float32))
        gp = jnp.concatenate(gs, axis=1) + b2b[...].astype(jnp.float32).reshape(1, D)
        gate = gp * jax.nn.sigmoid(gp)
        sa = so[0:2] + so[2:4]
        o_ref[...] = (xf + sa * gate[0:2]).astype(o_ref.dtype)

    def f(A_x, A_k_cache, A_v_cache, A_wq, A_wo, B_x, B_w1, B_b1, B_w2, B_b2):
        B, S, D = A_x.shape
        HD = A_wq.shape[1]
        F = B_w1.shape[1]
        HKV, DH = A_k_cache.shape[1], A_k_cache.shape[3]
        bf = jnp.bfloat16
        W = 4096
        out = pl.pallas_call(
            kern,
            out_shape=jax.ShapeDtypeStruct((B, D), A_x.dtype),
            in_specs=[pl.BlockSpec(memory_space=pl.ANY)] * 9,
            scratch_shapes=[
                pltpu.VMEM((B, D), bf), pltpu.VMEM((F,), bf), pltpu.VMEM((D,), bf),
                pltpu.VMEM((D, HD), bf), pltpu.VMEM((D, HD), bf), pltpu.VMEM((D, F), bf), pltpu.VMEM((D, F), bf),
                pltpu.VMEM((R, 8, SR, DH), bf),
                pltpu.VMEM((HKV, 8, DH), jnp.float32),
                pltpu.VMEM((2, W // SR, 4, 8, SR), jnp.float32),
                pltpu.VMEM((8, F), jnp.float32),
                pltpu.SemaphoreType.DMA((3,)), pltpu.SemaphoreType.DMA((16,)), pltpu.SemaphoreType.DMA((R,)),
            ],
            compiler_params=pltpu.CompilerParams(vmem_limit_bytes=64 * 1024 * 1024, disable_bounds_checks=nobc),
        )(A_x.reshape(B, D), A_k_cache, A_v_cache, A_wq, A_wo.T, B_w1, B_b1, B_w2.T, B_b2)
        return out.reshape(B, S, D)
    return f


_f = build()


@jax.jit
def pallas_recurrent_scan__sliding_block_cached__dense_activation_gelu__decode_kernel(
    A_x, A_k_cache, A_v_cache, A_wq, A_wo, B_x, B_w1, B_b1, B_w2, B_b2):
    return _f(A_x, A_k_cache, A_v_cache, A_wq, A_wo, B_x, B_w1, B_b1, B_w2, B_b2)
```

```python
import functools, math
import jax
import jax.numpy as jnp
import jax.experimental.pallas as pl
import jax.experimental.pallas.tpu as pltpu

CH = 128
NT = (((1,), (1,)), ((), ()))
f32 = jnp.float32
bf16 = jnp.bfloat16


def build(SR=512, R=8, AHEAD=4, NSTR=6, NV1=2, WP=(0,), LO=None, VQ=1, scopes=False):
    def scope(n):
        return jax.named_scope(n) if scopes else (lambda f: f)
    def kern(x_hbm, k_hbm, v_hbm, wq_hbm, wot_hbm, w1_hbm, b1_hbm, w2t_hbm, b2_hbm, o_ref,
             xb, b1b, b2b, wqb, wob, w1b, w2b, kvb, q_scr, s_scr, h_scr, st, so_scr, g_scr, xn_scr,
             sem_s, sem_w, sem_kv):
        B, D = xb.shape
        _, HKV, SK, DH = k_hbm.shape
        W = min(4096, max(256, SK // 4))
        HD = wqb.shape[1]
        F = w1b.shape[1]
        NG = HKV // 2
        NS = W // SR
        LNS = NS.bit_length() - 1
        CPS = SR // CH
        base = SK - W
        c_exp = (DH ** -0.5) * math.log2(math.e)
        SROWS = D // NSTR
        NRB = SROWS // 8

        def wcopy(src, dst, sem, r, c, nc):
            sl = (pl.ds(pl.multiple_of(r, 8), 8), pl.ds(c if isinstance(c, int) else pl.multiple_of(c, nc), nc))
            return pltpu.make_async_copy(src.at[sl], dst.at[sl], sem)

        def issue_w(src, dst, sem, r0, parts, nstr=NSTR, srows=SROWS, pr=(0, 1)):
            nc = src.shape[1] // parts
            n = 0
            for p in range(parts):
                for s in range(nstr):
                    wcopy(src, dst, sem, s * srows + r0, p * nc, nc).start(priority=pr[n % len(pr)])
                    n += 1

        def kvcopies(t, g, s, slot):
            out = []
            for c in range(CPS):
                r = pl.multiple_of(base + s * SR + c * CH, CH)
                for u in range(4):
                    out.append(pltpu.make_async_copy(
                        (k_hbm, v_hbm)[t].at[u % 2, 2 * g + u // 2, pl.ds(r, CH), :],
                        kvb.at[slot, 4 * t + u, pl.ds(c * CH, CH), :], sem_kv.at[slot]))
            return out

        def start2(a, b_):
            for i in range(max(len(a), len(b_))):
                if i < len(a):
                    a[i].start(priority=0)
                if i < len(b_):
                    b_[i].start(priority=1)

        def wait_ref(d, sem):
            pltpu.make_async_copy(d, d, sem).wait()

        small = [pltpu.make_async_copy(a, b_, sem_s.at[i])
                 for i, (a, b_) in enumerate(((x_hbm, xb), (b1_hbm, b1b), (b2_hbm, b2b)))]
        for c in small:
            c.start()
        row128 = jax.lax.broadcasted_iota(jnp.int32, (8, DH), 0)

        def loop_a(i, _):
            issue_w(wq_hbm, wqb, sem_w.at[0], i * 8, 2)
        scope('la')(lambda: jax.lax.fori_loop(0, NRB, loop_a, None))()

        for c in small:
            c.wait()
        row = jax.lax.broadcasted_iota(jnp.int32, (8, D), 0)
        xf = xb[...].astype(f32)
        x8 = jnp.where(row % 2 == 0, jnp.broadcast_to(xf[0:1], (8, D)), jnp.broadcast_to(xf[1:2], (8, D)))
        mu = jnp.mean(x8, axis=-1, keepdims=True)
        xc = x8 - mu
        var = jnp.mean(xc * xc, axis=-1, keepdims=True)
        xn_scr[...] = xc / jnp.sqrt(var + 1e-5)
        h_scr[...] = jnp.broadcast_to(b1b[...].astype(f32).reshape(1, F), (8, F))
        g_scr[...] = jnp.broadcast_to(b2b[...].astype(f32).reshape(1, D), (8, D))
        so_scr[...] = jnp.zeros((8, D), f32)
        for u in range(4):
            st[0, u] = jnp.full((8, 128), -jnp.inf, f32)

        QI = 8
        QH = HKV // QI
        def loop_b(i, _):
            issue_w(w1_hbm, w1b, sem_w.at[1], i * 8, 3)
            ii = i - (NRB - QI)

            @pl.when(ii == 0)
            def _():
                wait_ref(wqb, sem_w.at[0])

            @pl.when(ii >= 0)
            @scope('q')
            def _():
                nc = QH * 2 * DH
                q = jnp.dot(xn_scr[...].astype(bf16), wqb[:, pl.ds(pl.multiple_of(ii * nc, nc), nc)],
                            preferred_element_type=f32)
                for h in range(QH):
                    q_scr[ii * QH + h] = jnp.where(row128 % 4 < 2, q[:, 2 * h * DH:(2 * h + 1) * DH],
                                                   q[:, (2 * h + 1) * DH:(2 * h + 2) * DH])
        jax.lax.fori_loop(0, NRB, loop_b, None)

        FC = 512
        NF = F // FC
        HC = 768
        DM = 512
        def loop_c(i, _):
            issue_w(w2t_hbm, w2b, sem_w.at[2], i * 8, 3, 8, DM // 8)
            ii = i - (DM // 64 - F // HC)

            @pl.when(ii == 0)
            def _():
                wait_ref(w1b, sem_w.at[1])

            @pl.when(ii >= 0)
            @scope('h')
            def _():
                sl = pl.ds(pl.multiple_of(ii * HC, HC), HC)
                hp = jnp.dot(xn_scr[...].astype(bf16), w1b[:, sl], preferred_element_type=f32) + h_scr[:, sl]
                h_scr[:, sl] = jax.nn.gelu(hp, approximate=True)
        jax.lax.fori_loop(0, DM // 64, loop_c, None)

        @scope('qk')
        def qk_step(g, s, slot):
            for u in range(4):
                qh = q_scr[2 * g + u // 2].astype(bf16)
                sc = jax.lax.dot_general(qh, kvb[slot, u], NT, preferred_element_type=f32) * c_exp
                s_scr[g & 1, s, u] = sc
                m = st[0, u]
                for j in range(SR // 128):
                    m = jnp.maximum(m, sc[:, j * 128:(j + 1) * 128])
                st[0, u] = m

        @scope('pv')
        def pv_step(g, s, slot):
            for u in range(4):
                p = jnp.exp2(s_scr[g & 1, s, u] - jnp.tile(st[1, u], (1, SR // 128)))
                ll = st[2, u]
                for j in range(SR // 128):
                    ll = ll + p[:, j * 128:(j + 1) * 128]
                st[2, u] = ll
                st[3, u] = st[3, u] + jnp.dot(p.astype(bf16), kvb[slot, 4 + u], preferred_element_type=f32)

        @scope('fin')
        def finish(g):
            o = [st[3, u] / jnp.sum(st[2, u], axis=-1, keepdims=True) for u in range(4)]
            parts = []
            for hh in range(2):
                comb = jnp.where(row128 % 2 == 0, o[2 * hh], o[2 * hh + 1])
                parts.append(jnp.where(row128 < 2, comb, 0.0))
                parts.append(jnp.where((row128 >= 2) & (row128 < 4), comb, 0.0))
            lhs = jnp.concatenate(parts, axis=1).astype(bf16)
            c0 = pl.multiple_of(g * 4 * DH, 4 * DH)
            so_scr[...] += jax.lax.dot_general(lhs, wob[:, pl.ds(c0, 4 * DH)], NT, preferred_element_type=f32)

        def newphase():
            for u in range(4):
                st[1, u] = jnp.broadcast_to(jnp.max(st[0, u], axis=-1, keepdims=True), (8, 128))
                st[0, u] = jnp.full((8, 128), -jnp.inf, f32)
                st[2, u] = jnp.zeros((8, 128), f32)
                st[3, u] = jnp.zeros((8, 128), f32)

        P3, P4 = NS, NG * NS
        NSTEP = P4 + NS
        WI = 2 * NRB * 512 // (SR * 8)
        G0 = AHEAD

        def main(j, _):
            g, s, slot = j >> LNS, j & (NS - 1), j & (R - 1)

            @pl.when(j < P3)
            def _():
                if CPS == 4:
                    wl = [wcopy(wot_hbm, wob, sem_w.at[3], t * SROWS + ((s * 3 + a) >> 1) * 8, ((s * 3 + a) & 1) * (HD // 2), HD // 2)
                          for a in range(3) for t in range(NSTR)]
                else:
                    s2 = s >> 1
                    wl = [wcopy(wot_hbm, wob, sem_w.at[3], (t + (s & 1) * (NSTR // 2)) * SROWS + ((s2 * 3 + a) >> 1) * 8, ((s2 * 3 + a) & 1) * (HD // 2), HD // 2)
                          for a in range(3) for t in range(NSTR // 2)]
                start2(kvcopies(0, 0, s, slot), wl)

            @pl.when((j >= P3) & (j < P4))
            def _():
                start2(kvcopies(0, g, s, slot), kvcopies(1, g - 1, s, slot))

            @pl.when((j >= P4) & (j < NSTEP - NV1))
            def _():
                c = kvcopies(1, NG - 1, s, slot)
                start2(c[0::2], c[1::2])

            if NV1:
                @pl.when((j >= NSTEP - NV1) & (j < NSTEP))
                def _():
                    start2(*([], kvcopies(1, NG - 1, s, slot))[::(1 if VQ else -1)])

            @pl.when(j == NSTEP)
            def _():
                if LO is None:
                    issue_w(w2t_hbm, w2b, sem_w.at[4], DM, 3, (D - DM) // 8, 8, WP)
                else:
                    parts, ns = LO
                    tot = parts * (D - DM) // 8
                    n = 0
                    for a in range(tot // ns):
                        for t in range(ns):
                            rb, p = divmod(t * (tot // ns) + a, parts)
                            wcopy(w2t_hbm, w2b, sem_w.at[4], DM + 8 * rb, p * (F // parts), F // parts).start(priority=WP[n % len(WP)])
                            n += 1

            jg = j - G0

            @pl.when(jg == 0)
            def _():
                wait_ref(w2b.at[pl.ds(0, DM)], sem_w.at[2])

            @pl.when((jg >= 0) & (jg < NF))
            @scope('g')
            def _():
                sl = pl.ds(pl.multiple_of(jg * FC, FC), FC)
                g_scr[:, :DM] += jax.lax.dot_general(h_scr[:, sl].astype(bf16), w2b[:DM, sl], NT, preferred_element_type=f32)

            @pl.when(jg == NF)
            def _():
                gp = g_scr[:, :DM]
                g_scr[:, :DM] = gp * jax.nn.sigmoid(gp)
                wait_ref(wob, sem_w.at[3])

            i = j - AHEAD
            g, s, slot = i >> LNS, i & (NS - 1), i & (R - 1)

            @pl.when((i >= 0) & (i < P3))
            def _():
                wait_ref(kvb.at[slot, pl.ds(0, 4)], sem_kv.at[slot])

            @pl.when((i >= P3) & (i < P4))
            def _():
                wait_ref(kvb.at[slot], sem_kv.at[slot])

            @pl.when(i >= P4)
            def _():
                wait_ref(kvb.at[slot, pl.ds(4, 4)], sem_kv.at[slot])

            @pl.when((i >= 0) & (i < P4))
            def _():
                qk_step(g, s, slot)

            @pl.when(i >= P3)
            def _():
                pv_step(g - 1, s, slot)

            @pl.when((i >= P3) & (s == NS - 1))
            def _():
                finish(g - 1)

            @pl.when((i >= 0) & (i < P4) & (s == NS - 1))
            def _():
                newphase()

        jax.lax.fori_loop(0, NSTEP + AHEAD, main, None)
        so = so_scr[...]
        sa = so[0:2] + so[2:4]
        xf = xb[...].astype(f32)
        o_ref[:, :DM] = (xf[:, :DM] + sa[:, :DM] * g_scr[0:2, :DM]).astype(o_ref.dtype)
        hb = h_scr[...].astype(bf16)
        scope('wl')(lambda: wait_ref(w2b.at[pl.ds(DM, D - DM)], sem_w.at[4]))()
        gp = g_scr[:, DM:] + jax.lax.dot_general(hb, w2b[DM:, :], NT, preferred_element_type=f32)
        gp = gp[0:2]
        o_ref[:, DM:] = (xf[:, DM:] + sa[:, DM:] * (gp * jax.nn.sigmoid(gp))).astype(o_ref.dtype)

    def f(A_x, A_k_cache, A_v_cache, A_wq, A_wo, B_x, B_w1, B_b1, B_w2, B_b2):
        B, S, D = A_x.shape
        HD = A_wq.shape[1]
        F = B_w1.shape[1]
        HKV, DH = A_k_cache.shape[1], A_k_cache.shape[3]
        W = 4096
        out = pl.pallas_call(
            kern,
            out_shape=jax.ShapeDtypeStruct((B, D), A_x.dtype),
            in_specs=[pl.BlockSpec(memory_space=pl.ANY)] * 9,
            scratch_shapes=[
                pltpu.VMEM((B, D), bf16), pltpu.VMEM((F,), bf16), pltpu.VMEM((D,), bf16),
                pltpu.VMEM((D, HD), bf16), pltpu.VMEM((D, HD), bf16), pltpu.VMEM((D, F), bf16), pltpu.VMEM((D, F), bf16),
                pltpu.VMEM((R, 8, SR, DH), bf16),
                pltpu.VMEM((HKV, 8, DH), f32),
                pltpu.VMEM((2, W // SR, 4, 8, SR), f32),
                pltpu.VMEM((8, F), f32),
                pltpu.VMEM((4, 4, 8, DH), f32),
                pltpu.VMEM((8, D), f32), pltpu.VMEM((8, D), f32), pltpu.VMEM((8, D), f32),
                pltpu.SemaphoreType.DMA((3,)), pltpu.SemaphoreType.DMA((5,)), pltpu.SemaphoreType.DMA((R,)),
            ],
            compiler_params=pltpu.CompilerParams(vmem_limit_bytes=64 * 1024 * 1024, disable_bounds_checks=True),
        )(A_x.reshape(B, D), A_k_cache, A_v_cache, A_wq, A_wo.T, B_w1, B_b1, B_w2.T, B_b2)
        return out.reshape(B, S, D)
    return f


_f = build(NV1=0, WP=(1,), LO=(3, 1))


@jax.jit
def pallas_recurrent_scan__sliding_block_cached__dense_activation_gelu__decode_kernel(
    A_x, A_k_cache, A_v_cache, A_wq, A_wo, B_x, B_w1, B_b1, B_w2, B_b2):
    return _f(A_x, A_k_cache, A_v_cache, A_wq, A_wo, B_x, B_w1, B_b1, B_w2, B_b2)
```

```python
import math
import jax
import jax.numpy as jnp
import jax.experimental.pallas as pl
import jax.experimental.pallas.tpu as pltpu

CH = 128
SR = 512
R = 8
NT = (((1,), (1,)), ((), ()))
f32 = jnp.float32
bf16 = jnp.bfloat16


def build(AHEAD=4, NSTR=6, DM=512, WP=(1,), scopes=False, HACK=(0, 0), hmode=False):
    def scope(n):
        return jax.named_scope(n) if scopes else (lambda f: f)

    def kern(x_hbm, k_hbm, v_hbm, wq_hbm, wot_hbm, w1_hbm, b1_hbm, w2t_hbm, b2_hbm, o_ref,
             xb, b1b, b2b, wqb, wob, w1b, w2b, kvb, q_scr, s_scr, h_scr, st, so_scr, g_scr, xn_scr, o_scr,
             sem_s, sem_w, sem_kv):
        B, D = xb.shape
        _, HKV, SK, DH = k_hbm.shape
        W = min(4096, max(256, SK // 4))
        HD = wqb.shape[1]
        F = w1b.shape[1]
        NG = HKV // 2
        NS = W // SR
        LNS = NS.bit_length() - 1
        CPS = SR // CH
        base = SK - W
        c_exp = (DH ** -0.5) * math.log2(math.e)
        SROWS = D // NSTR
        NRB = SROWS // 8

        def wcopies(src, dst, sem, r0, parts, nstr=NSTR, srows=SROWS):
            nc = src.shape[1] // parts
            out = []
            for p in range(parts):
                for s in range(nstr):
                    r = s * srows + r0
                    sl = (pl.ds(r if isinstance(r, int) else pl.multiple_of(r, 8), 8), pl.ds(p * nc, nc))
                    out.append(pltpu.make_async_copy(src.at[sl], dst.at[sl], sem))
            return out

        def kvcopies(t, g, s, slot):
            out = []
            for c in range(CPS):
                r = pl.multiple_of(base - HACK[t] + s * SR + c * CH, 16)
                for u in range(4):
                    bb, hh = (g & 1, 4 * (g >> 1) + u) if hmode else (u % 2, 2 * g + u // 2)
                    out.append(pltpu.make_async_copy(
                        (k_hbm, v_hbm)[t].at[bb, hh, pl.ds(r, CH), :],
                        kvb.at[slot, 4 * t + u, pl.ds(c * CH, CH), :], sem_kv.at[slot]))
            return out

        def start2(a, b_):
            for i in range(max(len(a), len(b_))):
                if i < len(a):
                    a[i].start(priority=0)
                if i < len(b_):
                    b_[i].start(priority=1)

        def start1(c):
            start2(c[0::2], c[1::2])

        def wait_ref(d, sem):
            pltpu.make_async_copy(d, d, sem).wait()

        small = [pltpu.make_async_copy(a, b_, sem_s.at[i])
                 for i, (a, b_) in enumerate(((x_hbm, xb), (b1_hbm, b1b), (b2_hbm, b2b)))]
        for c in small:
            c.start()
        row128 = jax.lax.broadcasted_iota(jnp.int32, (8, DH), 0)

        def loop_a(i, _):
            start1(wcopies(wq_hbm, wqb, sem_w.at[0], i * 8, 2))
        jax.lax.fori_loop(0, NRB, loop_a, None)

        for c in small:
            c.wait()
        row = jax.lax.broadcasted_iota(jnp.int32, (8, D), 0)
        xf = xb[...].astype(f32)
        x8 = jnp.where(row % 2 == 0, jnp.broadcast_to(xf[0:1], (8, D)), jnp.broadcast_to(xf[1:2], (8, D)))
        mu = jnp.mean(x8, axis=-1, keepdims=True)
        xc = x8 - mu
        var = jnp.mean(xc * xc, axis=-1, keepdims=True)
        xn_scr[...] = xc / jnp.sqrt(var + 1e-5)
        h_scr[...] = jnp.broadcast_to(b1b[...].astype(f32).reshape(1, F), (8, F))
        g_scr[...] = jnp.broadcast_to(b2b[...].astype(f32).reshape(1, D), (8, D))
        so_scr[...] = jnp.zeros(so_scr.shape, f32)
        for u in range(4):
            st[0, u] = jnp.full((8, 128), -jnp.inf, f32)

        QI = 8
        QH = HKV // QI

        def loop_b(i, _):
            start1(wcopies(w1_hbm, w1b, sem_w.at[1], i * 8, 3))
            ii = i - (NRB - QI)

            @pl.when(ii == 0)
            def _():
                wait_ref(wqb, sem_w.at[0])

            @pl.when(ii >= 0)
            @scope('q')
            def _():
                nc = QH * 2 * DH
                q = jnp.dot(xn_scr[...].astype(bf16), wqb[:, pl.ds(pl.multiple_of(ii * nc, nc), nc)],
                            preferred_element_type=f32)
                for h in range(QH):
                    q_scr[ii * QH + h] = jnp.where(row128 % 4 < 2, q[:, 2 * h * DH:(2 * h + 1) * DH],
                                                   q[:, (2 * h + 1) * DH:(2 * h + 2) * DH])
        jax.lax.fori_loop(0, NRB, loop_b, None)

        FC = 512
        NF = F // FC

        def loop_c(i, _):
            start1(wcopies(w2t_hbm, w2b, sem_w.at[2], i * 8, 3))
            ii = i - (NRB - NF)

            @pl.when(ii == 0)
            def _():
                wait_ref(w1b, sem_w.at[1])

            @pl.when(ii >= 0)
            @scope('h')
            def _():
                sl = pl.ds(pl.multiple_of(ii * FC, FC), FC)
                hp = jnp.dot(xn_scr[...].astype(bf16), w1b[:, sl], preferred_element_type=f32) + h_scr[:, sl]
                h_scr[:, sl] = jax.nn.gelu(hp, approximate=True)
        jax.lax.fori_loop(0, NRB, loop_c, None)

        @scope('qk')
        def qk_step(g, s, slot):
            for u in range(4):
                qh = q_scr[2 * g + u // 2].astype(bf16)
                sc = jax.lax.dot_general(qh, kvb[slot, u], NT, preferred_element_type=f32) * c_exp
                s_scr[g & 1, s, u] = sc
                m = st[0, u]
                for j in range(SR // 128):
                    m = jnp.maximum(m, sc[:, j * 128:(j + 1) * 128])
                st[0, u] = m

        @scope('pv')
        def pv_step(g, s, slot):
            for u in range(4):
                p = jnp.exp2(s_scr[g & 1, s, u] - jnp.tile(st[1, u], (1, SR // 128)))
                ll = st[2, u]
                for j in range(SR // 128):
                    ll = ll + p[:, j * 128:(j + 1) * 128]
                st[2, u] = ll
                st[3, u] = st[3, u] + jnp.dot(p.astype(bf16), kvb[slot, 4 + u], preferred_element_type=f32)

        @scope('fin')
        def finish(g):
            o = [st[3, u] / jnp.sum(st[2, u], axis=-1, keepdims=True) for u in range(4)]
            parts = []
            for hh in range(2):
                comb = jnp.where(row128 % 2 == 0, o[2 * hh], o[2 * hh + 1])
                parts.append(jnp.where(row128 < 2, comb, 0.0))
                parts.append(jnp.where((row128 >= 2) & (row128 < 4), comb, 0.0))
            lhs = jnp.concatenate(parts, axis=1)
            c0 = pl.ds(pl.multiple_of(g * 4 * DH, 4 * DH), 4 * DH)
            o_scr[:, c0] = lhs
            so_scr[...] += jax.lax.dot_general(lhs.astype(bf16), wob[:DM, c0], NT, preferred_element_type=f32)

        def newphase():
            for u in range(4):
                st[1, u] = jnp.broadcast_to(jnp.max(st[0, u], axis=-1, keepdims=True), (8, 128))
                st[0, u] = jnp.full((8, 128), -jnp.inf, f32)
                st[2, u] = jnp.zeros((8, 128), f32)
                st[3, u] = jnp.zeros((8, 128), f32)

        P3, P4 = NS, NG * NS
        NSTEP = P4 + NS

        def main(j, _):
            g, s, slot = j >> LNS, j & (NS - 1), j & (R - 1)

            @pl.when(j < P3)
            def _():
                start2(kvcopies(0, 0, s, slot),
                       wcopies(wot_hbm, wob, sem_w.at[3], s * 8, 2, DM // (8 * NS), 8 * NS))

            @pl.when((j >= P3) & (j < P4))
            def _():
                start2(kvcopies(0, g, s, slot), kvcopies(1, g - 1, s, slot))

            @pl.when((j >= P4) & (j < NSTEP))
            def _():
                start1(kvcopies(1, NG - 1, s, slot))

            @pl.when(j == NSTEP)
            def _():
                n = 0
                for r in range(DM, D, 8):
                    for c in wcopies(wot_hbm, wob, sem_w.at[4], r, 2, 1, 0):
                        c.start(priority=WP[n % len(WP)])
                        n += 1

            i = j - AHEAD
            g, s, slot = i >> LNS, i & (NS - 1), i & (R - 1)

            @pl.when(i == 0)
            def _():
                wait_ref(w2b, sem_w.at[2])

            @pl.when((i >= 0) & (i < NF))
            @scope('g')
            def _():
                sl = pl.ds(pl.multiple_of(i * FC, FC), FC)
                g_scr[...] += jax.lax.dot_general(h_scr[:, sl].astype(bf16), w2b[:, sl], NT, preferred_element_type=f32)

            @pl.when(i == NF)
            def _():
                gp = g_scr[...]
                g_scr[...] = gp * jax.nn.sigmoid(gp)
                wait_ref(wob.at[pl.ds(0, DM)], sem_w.at[3])

            @pl.when((i >= 0) & (i < P3))
            def _():
                wait_ref(kvb.at[slot, pl.ds(0, 4)], sem_kv.at[slot])

            @pl.when((i >= P3) & (i < P4))
            def _():
                wait_ref(kvb.at[slot], sem_kv.at[slot])

            @pl.when(i >= P4)
            def _():
                wait_ref(kvb.at[slot, pl.ds(4, 4)], sem_kv.at[slot])

            @pl.when((i >= 0) & (i < P4))
            def _():
                qk_step(g, s, slot)

            @pl.when(i >= P3)
            def _():
                pv_step(g - 1, s, slot)

            @pl.when((i >= P3) & (s == NS - 1))
            def _():
                finish(g - 1)

            @pl.when((i >= 0) & (i < P4) & (s == NS - 1))
            def _():
                newphase()

        jax.lax.fori_loop(0, NSTEP + AHEAD, main, None)
        so = so_scr[...]
        xf = xb[...].astype(f32)
        o_ref[:, :DM] = (xf[:, :DM] + (so[0:2] + so[2:4]) * g_scr[0:2, :DM]).astype(o_ref.dtype)
        ob = o_scr[...].astype(bf16)
        scope('wl')(lambda: wait_ref(wob.at[pl.ds(DM, D - DM)], sem_w.at[4]))()
        so = jax.lax.dot_general(ob, wob[DM:, :], NT, preferred_element_type=f32)
        o_ref[:, DM:] = (xf[:, DM:] + (so[0:2] + so[2:4]) * g_scr[0:2, DM:]).astype(o_ref.dtype)

    def f(A_x, A_k_cache, A_v_cache, A_wq, A_wo, B_x, B_w1, B_b1, B_w2, B_b2):
        B, S, D = A_x.shape
        HD = A_wq.shape[1]
        F = B_w1.shape[1]
        HKV, DH = A_k_cache.shape[1], A_k_cache.shape[3]
        W = 4096
        out = pl.pallas_call(
            kern,
            out_shape=jax.ShapeDtypeStruct((B, D), A_x.dtype),
            in_specs=[pl.BlockSpec(memory_space=pl.ANY)] * 9,
            scratch_shapes=[
                pltpu.VMEM((B, D), bf16), pltpu.VMEM((F,), bf16), pltpu.VMEM((D,), bf16),
                pltpu.VMEM((D, HD), bf16), pltpu.VMEM((D, HD), bf16), pltpu.VMEM((D, F), bf16), pltpu.VMEM((D, F), bf16),
                pltpu.VMEM((R, 8, SR, DH), bf16),
                pltpu.VMEM((HKV, 8, DH), f32),
                pltpu.VMEM((2, W // SR, 4, 8, SR), f32),
                pltpu.VMEM((8, F), f32),
                pltpu.VMEM((4, 4, 8, DH), f32),
                pltpu.VMEM((8, DM), f32), pltpu.VMEM((8, D), f32), pltpu.VMEM((8, D), f32), pltpu.VMEM((8, HD), f32),
                pltpu.SemaphoreType.DMA((3,)), pltpu.SemaphoreType.DMA((5,)), pltpu.SemaphoreType.DMA((R,)),
            ],
            compiler_params=pltpu.CompilerParams(vmem_limit_bytes=64 * 1024 * 1024, disable_bounds_checks=True,
                                                 disable_semaphore_checks=True),
        )(A_x.reshape(B, D), A_k_cache, A_v_cache, A_wq, A_wo.T, B_w1, B_b1, B_w2.T, B_b2)
        return out.reshape(B, S, D)
    return f


_f = build()


@jax.jit
def pallas_recurrent_scan__sliding_block_cached__dense_activation_gelu__decode_kernel(
    A_x, A_k_cache, A_v_cache, A_wq, A_wo, B_x, B_w1, B_b1, B_w2, B_b2):
    return _f(A_x, A_k_cache, A_v_cache, A_wq, A_wo, B_x, B_w1, B_b1, B_w2, B_b2)
```

```python
import math
import jax
import jax.numpy as jnp
import jax.experimental.pallas as pl
import jax.experimental.pallas.tpu as pltpu

CH = 128
SR = 512
R = 8
NT = (((1,), (1,)), ((), ()))
f32 = jnp.float32
bf16 = jnp.bfloat16


def build(AHEAD=5, NSTR=6, DM=512, WP=(1,), scopes=False, VS=64):
    def scope(n):
        return jax.named_scope(n) if scopes else (lambda f: f)

    def kern(x_hbm, k_hbm, v_hbm, wq_hbm, wot_hbm, w1_hbm, b1_hbm, w2t_hbm, b2_hbm, o_ref,
             xb, b1b, b2b, wqb, wob, w1b, w2b, kvb, q_scr, s_scr, h_scr, st, so_scr, g_scr, xn_scr, o_scr,
             sem_s, sem_w, sem_kv):
        B, D = xb.shape
        _, HKV, SK, DH = k_hbm.shape
        W = min(4096, max(256, SK // 4))
        HD = wqb.shape[1]
        F = w1b.shape[1]
        NG = HKV // 2
        NS = W // SR
        LNS = NS.bit_length() - 1
        CPS = SR // CH
        base = SK - W
        c_exp = (DH ** -0.5) * math.log2(math.e)
        SROWS = D // NSTR
        NRB = SROWS // 8

        def wcopies(src, dst, sem, r0, parts, nstr=NSTR, srows=SROWS):
            nc = src.shape[1] // parts
            out = []
            for p in range(parts):
                for s in range(nstr):
                    r = s * srows + r0
                    sl = (pl.ds(r if isinstance(r, int) else pl.multiple_of(r, 8), 8), pl.ds(p * nc, nc))
                    out.append(pltpu.make_async_copy(src.at[sl], dst.at[sl], sem))
            return out

        def units(g):
            h0 = ((0x76440220 >> (4 * g)) & 15) * 2
            b0 = (0b00101100 >> g) & 1
            return [(jnp.where(g < 6, b0, u >> 1), h0 + jnp.where(g < 6, u, u & 1)) for u in range(4)]

        def kvcopies(t, g, s, off, n):
            r = pl.multiple_of(s * SR + off, 8)
            return [pltpu.make_async_copy(
                (k_hbm, v_hbm)[t].at[bb, hh, pl.ds(base + r, n), :],
                kvb.at[4 * t + u, pl.ds(r, n), :], sem_kv.at[s]) for u, (bb, hh) in enumerate(units(g))]

        def issue_kv(gk, gv, s):
            def go(c, voff, vn):
                v = kvcopies(1, gv, s, voff, vn)
                if gk is None:
                    start1(v)
                else:
                    start2(kvcopies(0, gk, s, c * CH, CH), v)

            @pl.when(s == 0)
            def _():
                start1(kvcopies(1, gv, s, 0, VS))
            for c in range(CPS - 1):
                go(c, VS + c * CH, CH)
            c = CPS - 1
            pl.when(s < NS - 1)(lambda: go(c, VS + c * CH, CH))
            pl.when(s == NS - 1)(lambda: go(c, VS + c * CH, CH - VS))

        def wait_v(s):
            for cond, n in ((s == 0, SR + VS), ((s > 0) & (s < NS - 1), SR), (s == NS - 1, SR - VS)):
                pl.when(cond)(lambda: wait_ref(kvb.at[pl.ds(4, 4), pl.ds(0, n)], sem_kv.at[s]))

        def start2(a, b_):
            for i in range(max(len(a), len(b_))):
                if i < len(a):
                    a[i].start(priority=0)
                if i < len(b_):
                    b_[i].start(priority=1)

        def start1(c):
            start2(c[0::2], c[1::2])

        def wait_ref(d, sem):
            pltpu.make_async_copy(d, d, sem).wait()

        small = [pltpu.make_async_copy(a, b_, sem_s.at[i])
                 for i, (a, b_) in enumerate(((x_hbm, xb), (b1_hbm, b1b), (b2_hbm, b2b)))]
        for c in small:
            c.start()
        row128 = jax.lax.broadcasted_iota(jnp.int32, (8, DH), 0)

        def loop_a(i, _):
            start1(wcopies(wq_hbm, wqb, sem_w.at[0], i * 8, 2))
        jax.lax.fori_loop(0, NRB, loop_a, None)

        for c in small:
            c.wait()
        row = jax.lax.broadcasted_iota(jnp.int32, (8, D), 0)
        xf = xb[...].astype(f32)
        x8 = jnp.where(row % 2 == 0, jnp.broadcast_to(xf[0:1], (8, D)), jnp.broadcast_to(xf[1:2], (8, D)))
        mu = jnp.mean(x8, axis=-1, keepdims=True)
        xc = x8 - mu
        var = jnp.mean(xc * xc, axis=-1, keepdims=True)
        xn_scr[...] = xc / jnp.sqrt(var + 1e-5)
        h_scr[...] = jnp.broadcast_to(b1b[...].astype(f32).reshape(1, F), (8, F))
        g_scr[...] = jnp.broadcast_to(b2b[...].astype(f32).reshape(1, D), (8, D))
        so_scr[...] = jnp.zeros(so_scr.shape, f32)
        o_scr[...] = jnp.zeros(o_scr.shape, f32)
        for u in range(4):
            st[0, u] = jnp.full((8, 128), -jnp.inf, f32)

        QI = 8
        QH = HKV // QI

        def loop_b(i, _):
            start1(wcopies(w1_hbm, w1b, sem_w.at[1], i * 8, 3))
            ii = i - (NRB - QI)

            @pl.when(ii == 0)
            def _():
                wait_ref(wqb, sem_w.at[0])

            @pl.when(ii >= 0)
            @scope('q')
            def _():
                nc = QH * 2 * DH
                q = jnp.dot(xn_scr[...].astype(bf16), wqb[:, pl.ds(pl.multiple_of(ii * nc, nc), nc)],
                            preferred_element_type=f32)
                for h in range(QH):
                    q_scr[ii * QH + h] = jnp.where(row128 % 4 < 2, q[:, 2 * h * DH:(2 * h + 1) * DH],
                                                   q[:, (2 * h + 1) * DH:(2 * h + 2) * DH])
        jax.lax.fori_loop(0, NRB, loop_b, None)

        FC = 512
        NF = F // FC

        def loop_c(i, _):
            start1(wcopies(w2t_hbm, w2b, sem_w.at[2], i * 8, 3))
            ii = i - (NRB - NF)

            @pl.when(ii == 0)
            def _():
                wait_ref(w1b, sem_w.at[1])

            @pl.when(ii >= 0)
            @scope('h')
            def _():
                sl = pl.ds(pl.multiple_of(ii * FC, FC), FC)
                hp = jnp.dot(xn_scr[...].astype(bf16), w1b[:, sl], preferred_element_type=f32) + h_scr[:, sl]
                h_scr[:, sl] = jax.nn.gelu(hp, approximate=True)
        jax.lax.fori_loop(0, NRB, loop_c, None)

        @scope('qk')
        def qk_step(g, s):
            bh = units(g)
            for u in range(4):
                qh = q_scr[bh[u][1]].astype(bf16)
                sc = jax.lax.dot_general(qh, kvb[u, pl.ds(pl.multiple_of(s * SR, SR), SR)], NT, preferred_element_type=f32) * c_exp
                s_scr[g & 1, s, u] = sc
                m = st[0, u]
                for j in range(SR // 128):
                    m = jnp.maximum(m, sc[:, j * 128:(j + 1) * 128])
                st[0, u] = m

        @scope('pv')
        def pv_step(g, s):
            for u in range(4):
                p = jnp.exp2(s_scr[g & 1, s, u] - jnp.tile(st[1, u], (1, SR // 128)))
                ll = st[2, u]
                for j in range(SR // 128):
                    ll = ll + p[:, j * 128:(j + 1) * 128]
                st[2, u] = ll
                st[3, u] = st[3, u] + jnp.dot(p.astype(bf16), kvb[4 + u, pl.ds(pl.multiple_of(s * SR, SR), SR)], preferred_element_type=f32)

        @scope('fin')
        def finish(g):
            for u, (bb, hh) in enumerate(units(g)):
                o = st[3, u] / jnp.sum(st[2, u], axis=-1, keepdims=True)
                for r in range(2):
                    c = pl.ds(pl.multiple_of((2 * hh + r) * DH, DH), DH)
                    o_scr[:, c] = jnp.where(row128 == bb + 2 * r, o, o_scr[:, c])

        @scope('pr')
        def project(ch):
            c0 = pl.ds(pl.multiple_of(ch * 4 * DH, 4 * DH), 4 * DH)
            so_scr[...] += jax.lax.dot_general(o_scr[:, c0].astype(bf16), wob[:DM, c0], NT, preferred_element_type=f32)

        def newphase():
            for u in range(4):
                st[1, u] = jnp.broadcast_to(jnp.max(st[0, u], axis=-1, keepdims=True), (8, 128))
                st[0, u] = jnp.full((8, 128), -jnp.inf, f32)
                st[2, u] = jnp.zeros((8, 128), f32)
                st[3, u] = jnp.zeros((8, 128), f32)

        P3, P4 = NS, NG * NS
        NSTEP = P4 + NS

        def main(j, _):
            g, s = j >> LNS, j & (NS - 1)

            @pl.when(j < P3)
            def _():
                start2([d for c in range(CPS) for d in kvcopies(0, 0, s, c * CH, CH)],
                       wcopies(wot_hbm, wob, sem_w.at[3], s * 8, 2, DM // (8 * NS), 8 * NS))

            @pl.when((j >= P3) & (j < P4))
            def _():
                issue_kv(g, g - 1, s)

            @pl.when((j >= P4) & (j < NSTEP))
            def _():
                issue_kv(None, NG - 1, s)

            @pl.when(j == NSTEP)
            def _():
                n = 0
                for r in range(DM, D, 8):
                    for c in wcopies(wot_hbm, wob, sem_w.at[4], r, 2, 1, 0):
                        c.start(priority=WP[n % len(WP)])
                        n += 1

            i = j - AHEAD
            g, s = i >> LNS, i & (NS - 1)

            @pl.when(i == 0)
            def _():
                wait_ref(w2b, sem_w.at[2])

            @pl.when((i >= 0) & (i < NF))
            @scope('g')
            def _():
                sl = pl.ds(pl.multiple_of(i * FC, FC), FC)
                g_scr[...] += jax.lax.dot_general(h_scr[:, sl].astype(bf16), w2b[:, sl], NT, preferred_element_type=f32)

            @pl.when(i == NF)
            def _():
                gp = g_scr[...]
                g_scr[...] = gp * jax.nn.sigmoid(gp)
                wait_ref(wob.at[pl.ds(0, DM)], sem_w.at[3])

            @pl.when((i >= 0) & (i < P4))
            def _():
                wait_ref(kvb.at[pl.ds(0, 4), pl.ds(0, SR)], sem_kv.at[s])

            @pl.when(i >= P3)
            def _():
                wait_v(s)

            @pl.when((i >= 0) & (i < P4))
            def _():
                qk_step(g, s)

            @pl.when(i >= P3)
            def _():
                pv_step(g - 1, s)

            @pl.when((i >= P3) & (s == NS - 1))
            def _():
                finish(g - 1)

            @pl.when(((g == 5) | (g == NG)) & ((s < 3) | (s == NS - 1)))
            def _():
                project(jnp.minimum(s, 3) + jnp.where(g == NG, 4, 0))

            @pl.when((i >= 0) & (i < P4) & (s == NS - 1))
            def _():
                newphase()

        jax.lax.fori_loop(0, NSTEP + AHEAD, main, None)
        so = so_scr[...]
        xf = xb[...].astype(f32)
        o_ref[:, :DM] = (xf[:, :DM] + (so[0:2] + so[2:4]) * g_scr[0:2, :DM]).astype(o_ref.dtype)
        ob = o_scr[...].astype(bf16)
        scope('wl')(lambda: wait_ref(wob.at[pl.ds(DM, D - DM)], sem_w.at[4]))()
        so = jax.lax.dot_general(ob, wob[DM:, :], NT, preferred_element_type=f32)
        o_ref[:, DM:] = (xf[:, DM:] + (so[0:2] + so[2:4]) * g_scr[0:2, DM:]).astype(o_ref.dtype)

    def f(A_x, A_k_cache, A_v_cache, A_wq, A_wo, B_x, B_w1, B_b1, B_w2, B_b2):
        B, S, D = A_x.shape
        HD = A_wq.shape[1]
        F = B_w1.shape[1]
        HKV, DH = A_k_cache.shape[1], A_k_cache.shape[3]
        W = 4096
        out = pl.pallas_call(
            kern,
            out_shape=jax.ShapeDtypeStruct((B, D), A_x.dtype),
            in_specs=[pl.BlockSpec(memory_space=pl.ANY)] * 9,
            scratch_shapes=[
                pltpu.VMEM((B, D), bf16), pltpu.VMEM((F,), bf16), pltpu.VMEM((D,), bf16),
                pltpu.VMEM((D, HD), bf16), pltpu.VMEM((D, HD), bf16), pltpu.VMEM((D, F), bf16), pltpu.VMEM((D, F), bf16),
                pltpu.VMEM((8, W, DH), bf16),
                pltpu.VMEM((HKV, 8, DH), f32),
                pltpu.VMEM((2, W // SR, 4, 8, SR), f32),
                pltpu.VMEM((8, F), f32),
                pltpu.VMEM((4, 4, 8, DH), f32),
                pltpu.VMEM((8, DM), f32), pltpu.VMEM((8, D), f32), pltpu.VMEM((8, D), f32), pltpu.VMEM((8, HD), f32),
                pltpu.SemaphoreType.DMA((3,)), pltpu.SemaphoreType.DMA((5,)), pltpu.SemaphoreType.DMA((W // SR,)),
            ],
            compiler_params=pltpu.CompilerParams(vmem_limit_bytes=64 * 1024 * 1024, disable_bounds_checks=True,
                                                 disable_semaphore_checks=True),
        )(A_x.reshape(B, D), A_k_cache, A_v_cache, A_wq, A_wo.T, B_w1, B_b1, B_w2.T, B_b2)
        return out.reshape(B, S, D)
    return f


_f = build()


@jax.jit
def pallas_recurrent_scan__sliding_block_cached__dense_activation_gelu__decode_kernel(
    A_x, A_k_cache, A_v_cache, A_wq, A_wo, B_x, B_w1, B_b1, B_w2, B_b2):
    return _f(A_x, A_k_cache, A_v_cache, A_wq, A_wo, B_x, B_w1, B_b1, B_w2, B_b2)
```

```python
import math

import jax
import jax.numpy as jnp
import jax.experimental.pallas as pl
import jax.experimental.pallas.tpu as pltpu

CH = 128
SR = 512
VS = 64
AHEAD = 5
NU = 4
NSTR = 6
DM = 512
FC = 512
NT = (((1,), (1,)), ((), ()))
f32 = jnp.float32
bf16 = jnp.bfloat16


def _window(sk):
    return min(4096, max(256, sk // 4))


def _kernel(x_hbm, k_hbm, v_hbm, wq_hbm, wot_hbm, w1_hbm, b1_hbm, w2t_hbm, b2_hbm, o_ref,
            xb, b1b, b2b, wqb, wob, w1b, w2b, kvb,
            xn_scr, q_scr, s_scr, st, o_scr, so_scr, h_scr, g_scr,
            sem_s, sem_w, sem_kv):
    _, D = xb.shape
    _, HKV, SK, DH = k_hbm.shape
    F = w1b.shape[1]
    W = _window(SK)
    NG = 2 * HKV // NU
    NS = W // SR
    LNS = NS.bit_length() - 1
    CPS = SR // CH
    base = SK - W
    c_exp = (DH ** -0.5) * math.log2(math.e)
    SROWS = D // NSTR
    NRB = SROWS // 8
    NF = F // FC
    P3, P4 = NS, NG * NS
    NSTEP = P4 + NS
    assert (NG, NS) == (8, 8) and AHEAD <= NS - 2 and NF <= NRB and D % (8 * NSTR) == 0

    def start2(a, b):
        for i in range(max(len(a), len(b))):
            if i < len(a):
                a[i].start(priority=0)
            if i < len(b):
                b[i].start(priority=1)

    def start1(c):
        start2(c[0::2], c[1::2])

    def wait_ref(d, sem):
        pltpu.make_async_copy(d, d, sem).wait()

    def wcopies(src, dst, sem, r0, parts, nstr=NSTR, srows=SROWS):
        nc = src.shape[1] // parts
        out = []
        for p in range(parts):
            for t in range(nstr):
                r = t * srows + r0
                sl = (pl.ds(r if isinstance(r, int) else pl.multiple_of(r, 8), 8), pl.ds(p * nc, nc))
                out.append(pltpu.make_async_copy(src.at[sl], dst.at[sl], sem))
        return out

    def units(g):
        h0 = ((0x76440220 >> (4 * g)) & 15) * 2
        b0 = (0b00101100 >> g) & 1
        return [(jnp.where(g < 6, b0, u >> 1), h0 + jnp.where(g < 6, u, u & 1)) for u in range(NU)]

    def kvcopies(t, g, s, off, n):
        r = pl.multiple_of(s * SR + off, 8)
        return [pltpu.make_async_copy(
            (k_hbm, v_hbm)[t].at[bb, hh, pl.ds(base + r, n), :],
            kvb.at[NU * t + u, pl.ds(r, n), :], sem_kv.at[s]) for u, (bb, hh) in enumerate(units(g))]

    def issue_kv(gk, gv, s):
        def go(c, vn):
            v = kvcopies(1, gv, s, VS + c * CH, vn)
            if gk is None:
                start1(v)
            else:
                start2(kvcopies(0, gk, s, c * CH, CH), v)

        pl.when(s == 0)(lambda: start1(kvcopies(1, gv, s, 0, VS)))
        for c in range(CPS - 1):
            go(c, CH)
        pl.when(s < NS - 1)(lambda: go(CPS - 1, CH))
        pl.when(s == NS - 1)(lambda: go(CPS - 1, CH - VS))

    def wait_k(s):
        wait_ref(kvb.at[pl.ds(0, NU), pl.ds(pl.multiple_of(s * SR, SR), SR)], sem_kv.at[s])

    def wait_v(s):
        def go(r, n):
            wait_ref(kvb.at[pl.ds(NU, NU), pl.ds(r, n)], sem_kv.at[s])

        pl.when(s == 0)(lambda: go(0, SR + VS))
        pl.when((s > 0) & (s < NS - 1))(lambda: go(pl.multiple_of(s * SR + VS, 8), SR))
        pl.when(s == NS - 1)(lambda: go(W - SR + VS, SR - VS))

    small = [pltpu.make_async_copy(a, b, sem_s.at[i])
             for i, (a, b) in enumerate(((x_hbm, xb), (b1_hbm, b1b), (b2_hbm, b2b)))]
    for c in small:
        c.start()
    row128 = jax.lax.broadcasted_iota(jnp.int32, (8, DH), 0)

    def loop_a(i, _):
        start1(wcopies(wq_hbm, wqb, sem_w.at[0], i * 8, 2))
    jax.lax.fori_loop(0, NRB, loop_a, None)

    for c in small:
        c.wait()
    row = jax.lax.broadcasted_iota(jnp.int32, (8, D), 0)
    xf = xb[...].astype(f32)
    x8 = jnp.where(row % 2 == 0, jnp.broadcast_to(xf[0:1], (8, D)), jnp.broadcast_to(xf[1:2], (8, D)))
    xc = x8 - jnp.mean(x8, axis=-1, keepdims=True)
    var = jnp.mean(xc * xc, axis=-1, keepdims=True)
    xn_scr[...] = xc / jnp.sqrt(var + 1e-5)
    h_scr[...] = jnp.broadcast_to(b1b[...].astype(f32).reshape(1, F), (8, F))
    g_scr[...] = jnp.broadcast_to(b2b[...].astype(f32).reshape(1, D), (8, D))
    so_scr[...] = jnp.zeros(so_scr.shape, f32)
    o_scr[...] = jnp.zeros(o_scr.shape, f32)
    for u in range(NU):
        st[0, u] = jnp.full((8, DH), -jnp.inf, f32)

    QI = 8
    QH = HKV // QI

    def loop_b(i, _):
        start1(wcopies(w1_hbm, w1b, sem_w.at[1], i * 8, 3))
        ii = i - (NRB - QI)
        pl.when(ii == 0)(lambda: wait_ref(wqb, sem_w.at[0]))

        @pl.when(ii >= 0)
        def _():
            nc = QH * 2 * DH
            q = jnp.dot(xn_scr[...].astype(bf16), wqb[:, pl.ds(pl.multiple_of(ii * nc, nc), nc)],
                        preferred_element_type=f32)
            for h in range(QH):
                q_scr[ii * QH + h] = jnp.where(row128 % 4 < 2, q[:, 2 * h * DH:(2 * h + 1) * DH],
                                               q[:, (2 * h + 1) * DH:(2 * h + 2) * DH])
    jax.lax.fori_loop(0, NRB, loop_b, None)

    def loop_c(i, _):
        start1(wcopies(w2t_hbm, w2b, sem_w.at[2], i * 8, 3))
        ii = i - (NRB - NF)
        pl.when(ii == 0)(lambda: wait_ref(w1b, sem_w.at[1]))

        @pl.when(ii >= 0)
        def _():
            sl = pl.ds(pl.multiple_of(ii * FC, FC), FC)
            hp = jnp.dot(xn_scr[...].astype(bf16), w1b[:, sl], preferred_element_type=f32) + h_scr[:, sl]
            h_scr[:, sl] = jax.nn.gelu(hp, approximate=True)
    jax.lax.fori_loop(0, NRB, loop_c, None)

    def qk_step(g, s):
        rows = pl.ds(pl.multiple_of(s * SR, SR), SR)
        for u, (_, hh) in enumerate(units(g)):
            sc = jax.lax.dot_general(q_scr[hh].astype(bf16), kvb[u, rows], NT,
                                     preferred_element_type=f32) * c_exp
            s_scr[g & 1, s, u] = sc
            m = st[0, u]
            for j in range(SR // DH):
                m = jnp.maximum(m, sc[:, j * DH:(j + 1) * DH])
            st[0, u] = m

    def pv_step(g, s):
        rows = pl.ds(pl.multiple_of(s * SR, SR), SR)
        for u in range(NU):
            p = jnp.exp2(s_scr[g & 1, s, u] - jnp.tile(st[1, u], (1, SR // DH)))
            l = st[2, u]
            for j in range(SR // DH):
                l = l + p[:, j * DH:(j + 1) * DH]
            st[2, u] = l
            st[3, u] = st[3, u] + jnp.dot(p.astype(bf16), kvb[NU + u, rows], preferred_element_type=f32)

    def finish(g):
        for u, (bb, hh) in enumerate(units(g)):
            o = st[3, u] / jnp.sum(st[2, u], axis=-1, keepdims=True)
            for r in range(2):
                c = pl.ds(pl.multiple_of((2 * hh + r) * DH, DH), DH)
                o_scr[:, c] = jnp.where(row128 == bb + 2 * r, o, o_scr[:, c])

    def project(ch):
        c = pl.ds(pl.multiple_of(ch * 4 * DH, 4 * DH), 4 * DH)
        so_scr[...] += jax.lax.dot_general(o_scr[:, c].astype(bf16), wob[:DM, c], NT,
                                           preferred_element_type=f32)

    def next_group():
        for u in range(NU):
            st[1, u] = jnp.broadcast_to(jnp.max(st[0, u], axis=-1, keepdims=True), (8, DH))
            st[0, u] = jnp.full((8, DH), -jnp.inf, f32)
            st[2, u] = jnp.zeros((8, DH), f32)
            st[3, u] = jnp.zeros((8, DH), f32)

    def main(j, _):
        gj, sj = j >> LNS, j & (NS - 1)

        @pl.when(j < P3)
        def _():
            start2([d for c in range(CPS) for d in kvcopies(0, 0, sj, c * CH, CH)],
                   wcopies(wot_hbm, wob, sem_w.at[3], sj * 8, 2, DM // (8 * NS), 8 * NS))

        pl.when((j >= P3) & (j < P4))(lambda: issue_kv(gj, gj - 1, sj))
        pl.when((j >= P4) & (j < NSTEP))(lambda: issue_kv(None, NG - 1, sj))

        @pl.when(j == NSTEP)
        def _():
            for r in range(DM, D, 8):
                start2([], wcopies(wot_hbm, wob, sem_w.at[4], r, 2, 1, 0))

        i = j - AHEAD
        g, s = i >> LNS, i & (NS - 1)
        pl.when(i == 0)(lambda: wait_ref(w2b, sem_w.at[2]))

        @pl.when((i >= 0) & (i < NF))
        def _():
            sl = pl.ds(pl.multiple_of(i * FC, FC), FC)
            g_scr[...] += jax.lax.dot_general(h_scr[:, sl].astype(bf16), w2b[:, sl], NT,
                                              preferred_element_type=f32)

        @pl.when(i == NF)
        def _():
            gp = g_scr[...]
            g_scr[...] = gp * jax.nn.sigmoid(gp)
            wait_ref(wob.at[pl.ds(0, DM)], sem_w.at[3])

        has_k = (i >= 0) & (i < P4)
        has_v = i >= P3
        pl.when(has_k)(lambda: wait_k(s))
        pl.when(has_v)(lambda: wait_v(s))
        pl.when(has_k)(lambda: qk_step(g, s))
        pl.when(has_v)(lambda: pv_step(g - 1, s))
        pl.when(has_v & (s == NS - 1))(lambda: finish(g - 1))
        pl.when(((g == 5) | (g == NG)) & ((s < 3) | (s == NS - 1)))(
            lambda: project(jnp.minimum(s, 3) + jnp.where(g == NG, 4, 0)))
        pl.when(has_k & (s == NS - 1))(next_group)

    jax.lax.fori_loop(0, NSTEP + AHEAD, main, None)

    so = so_scr[...]
    xf = xb[...].astype(f32)
    o_ref[:, :DM] = (xf[:, :DM] + (so[0:2] + so[2:4]) * g_scr[0:2, :DM]).astype(o_ref.dtype)
    ob = o_scr[...].astype(bf16)
    wait_ref(wob.at[pl.ds(DM, D - DM)], sem_w.at[4])
    so = jax.lax.dot_general(ob, wob[DM:, :], NT, preferred_element_type=f32)
    o_ref[:, DM:] = (xf[:, DM:] + (so[0:2] + so[2:4]) * g_scr[0:2, DM:]).astype(o_ref.dtype)


@jax.jit
def pallas_recurrent_scan__sliding_block_cached__dense_activation_gelu__decode_kernel(
    A_x: jax.Array,
    A_k_cache: jax.Array,
    A_v_cache: jax.Array,
    A_wq: jax.Array,
    A_wo: jax.Array,
    B_x: jax.Array,
    B_w1: jax.Array,
    B_b1: jax.Array,
    B_w2: jax.Array,
    B_b2: jax.Array,
):
    del B_x
    B, S, D = A_x.shape
    HD = A_wq.shape[1]
    F = B_w1.shape[1]
    _, HKV, SK, DH = A_k_cache.shape
    W = _window(SK)
    assert (B, S) == (2, 1) and HD == 2 * HKV * DH
    out = pl.pallas_call(
        _kernel,
        out_shape=jax.ShapeDtypeStruct((B, D), A_x.dtype),
        in_specs=[pl.BlockSpec(memory_space=pl.ANY)] * 9,
        scratch_shapes=[
            pltpu.VMEM((B, D), bf16), pltpu.VMEM((F,), bf16), pltpu.VMEM((D,), bf16),
            pltpu.VMEM((D, HD), bf16), pltpu.VMEM((D, HD), bf16),
            pltpu.VMEM((D, F), bf16), pltpu.VMEM((D, F), bf16),
            pltpu.VMEM((2 * NU, W, DH), bf16),
            pltpu.VMEM((8, D), f32),
            pltpu.VMEM((HKV, 8, DH), f32),
            pltpu.VMEM((2, W // SR, NU, 8, SR), f32),
            pltpu.VMEM((4, NU, 8, DH), f32),
            pltpu.VMEM((8, HD), f32),
            pltpu.VMEM((8, DM), f32),
            pltpu.VMEM((8, F), f32),
            pltpu.VMEM((8, D), f32),
            pltpu.SemaphoreType.DMA((3,)),
            pltpu.SemaphoreType.DMA((5,)),
            pltpu.SemaphoreType.DMA((W // SR,)),
        ],
        compiler_params=pltpu.CompilerParams(
            vmem_limit_bytes=64 * 1024 * 1024,
            disable_bounds_checks=True,
            disable_semaphore_checks=True,
        ),
    )(A_x.reshape(B, D), A_k_cache, A_v_cache, A_wq, A_wo.T, B_w1, B_b1, B_w2.T, B_b2)
    return out.reshape(B, S, D)
```
